```python
import os as _os
_os.environ.setdefault("JAX_PLATFORMS", "cpu")
import jax
import jax.numpy as jnp

def _softmax(x, axis=-1):
    return jax.nn.softmax(x, axis=axis)
def _gelu(x):
    return jax.nn.gelu(x, approximate=True)
def _silu(x):
    return jax.nn.silu(x)
def _sigmoid(x):
    return jax.nn.sigmoid(x)
def _layernorm(x, axis=-1, eps=1e-5):
    m = jnp.mean(x, axis=axis, keepdims=True)
    v = jnp.var(x, axis=axis, keepdims=True)
    return (x - m) / jnp.sqrt(v + eps)
def _scatter_add(tgt, idx, src, axis=0):
    return tgt.at[idx].add(src)
def _segment_sum(src, seg, n):
    return jax.ops.segment_sum(src, seg, n)
class _Rng:
    def __init__(self, key):
        self._k = key
    def _next(self):
        self._k, sub = jax.random.split(self._k)
        return sub
    def normal(self, shape):
        return jax.random.normal(self._next(), shape, dtype=jnp.bfloat16)
    def randint(self, lo, hi, shape):
        return jax.random.randint(self._next(), shape, lo, hi, dtype=jnp.int32)
    def uniform(self, shape, lo=0.0, hi=1.0):
        return jax.random.uniform(self._next(), shape, jnp.bfloat16, lo, hi)
    def permutation(self, n):
        return jax.random.permutation(self._next(), n)


kernel_name = 'standalone__instancenorm__sampling'

def setup_inputs():
    _rng = _Rng(jax.random.key(int.from_bytes(__import__("os").urandom(4), "little")))
    _w = (lambda a: (lambda t: t.astype(jnp.bfloat16) if jnp.issubdtype(t.dtype, jnp.floating) else t)(jnp.asarray(a)))
    B, C, H, W = 16, 640, 16, 32
    return {
        "x": _w((lambda *s: _rng.normal(s) * 0.05)(B, C, H, W)),
        "g": _w((lambda *s: _rng.normal(s) * 0.05)(C) + 1.0),
        "b": _w((lambda *s: _rng.normal(s) * 0.05)(C)),
    }

def reference(x, g, b):
    mu = x.mean(axis=(-2, -1), keepdims=True)
    var = ((x - mu) * (x - mu)).mean(axis=(-2, -1), keepdims=True)
    xhat = (x - mu) / jnp.sqrt(var + 1e-5)
    return xhat * g.reshape(1, -1, 1, 1) + b.reshape(1, -1, 1, 1)
```

```python
import jax
import jax.numpy as jnp
import jax.experimental.pallas as pl
import jax.experimental.pallas.tpu as pltpu

_EPS = 1e-5


def _read_chunks(num_batches, rows):
    if num_batches < 4 or num_batches % 2 or rows % 128:
        return (rows,) * num_batches
    tail = (rows * 5 // 8) // 16 * 16
    return ((2 * rows,) * ((num_batches - 4) // 2)
            + (rows, rows, 2 * rows - tail, tail))


@jax.jit
def pallas_standalone__instancenorm__sampling_kernel(
    x: jax.Array,
    g: jax.Array,
    b: jax.Array,
):
    B, C, H, W = x.shape
    R = H * W
    N = B * R
    assert B >= 2 and R % 16 == 0

    read_rows = _read_chunks(B, R)
    nr = len(read_rows)
    roff = [sum(read_rows[:i]) for i in range(nr)]
    wait_at = [off // R for off in roff]
    k = wait_at[nr - 2]
    assert sum(read_rows) == N and 0 < k < wait_at[nr - 1]

    def kernel(x_hbm, g_hbm, b_hbm, o_hbm, xbuf, obuf, gbuf, bbuf, sems):
        ins = [
            pltpu.make_async_copy(
                x_hbm.at[pl.ds(roff[i], read_rows[i])],
                xbuf.at[pl.ds(roff[i], read_rows[i])],
                sems.at[i % 2])
            for i in range(nr)
        ]
        out_head = pltpu.make_async_copy(
            obuf.at[pl.ds(0, k * R)], o_hbm.at[pl.ds(0, k * R)],
            sems.at[(nr - 2) % 2])
        out_tail = pltpu.make_async_copy(
            obuf.at[pl.ds(k * R, N - k * R)], o_hbm.at[pl.ds(k * R, N - k * R)],
            sems.at[(nr - 1) % 2])
        copy_g = pltpu.make_async_copy(g_hbm, gbuf, sems.at[0])
        copy_b = pltpu.make_async_copy(b_hbm, bbuf, sems.at[0])

        ins[0].start()
        copy_g.start()
        copy_b.start()
        ins[1].start()

        def normalize(bi):
            gamma = gbuf[...].astype(jnp.float32).reshape(1, C)
            beta = bbuf[...].astype(jnp.float32).reshape(1, C)
            base = pl.multiple_of(bi * R, R)
            xb = xbuf[pl.ds(base, R), :].astype(jnp.float32)
            mu = jnp.sum(xb, axis=0, keepdims=True) * (1.0 / R)
            d = xb - mu
            var = jnp.sum(d * d, axis=0, keepdims=True) * (1.0 / R)
            scale = jax.lax.rsqrt(var + _EPS) * gamma
            obuf[pl.ds(base, R), :] = (d * scale + beta).astype(obuf.dtype)

        def body(bi, carry):
            for i in range(nr):
                @pl.when(bi == wait_at[i])
                def _():
                    if i == 0:
                        copy_g.wait()
                        copy_b.wait()
                    ins[i].wait()
                    if i + 2 < nr:
                        ins[i + 2].start()
                    if i == nr - 2:
                        out_head.start()
            normalize(bi)
            return carry

        jax.lax.fori_loop(0, B, body, 0)
        out_tail.start()
        out_head.wait()
        out_tail.wait()

    xt = jnp.transpose(x, (0, 2, 3, 1)).reshape(N, C)
    out = pl.pallas_call(
        kernel,
        in_specs=[pl.BlockSpec(memory_space=pl.ANY)] * 3,
        out_specs=pl.BlockSpec(memory_space=pl.ANY),
        out_shape=jax.ShapeDtypeStruct((N, C), x.dtype),
        scratch_shapes=[
            pltpu.VMEM((N, C), x.dtype),
            pltpu.VMEM((N, C), x.dtype),
            pltpu.VMEM((C,), g.dtype),
            pltpu.VMEM((C,), b.dtype),
            pltpu.SemaphoreType.DMA((2,)),
        ],
        compiler_params=pltpu.CompilerParams(vmem_limit_bytes=64 * 1024 * 1024),
    )(xt, g, b)
    return jnp.transpose(out.reshape(B, H, W, C), (0, 3, 1, 2))
```

```python
import jax
import jax.numpy as jnp
import jax.experimental.pallas as pl
import jax.experimental.pallas.tpu as pltpu

_EPS = 1e-5
_BLK = 32


@jax.jit
def pallas_standalone__instancenorm__sampling_kernel(
    x: jax.Array,
    g: jax.Array,
    b: jax.Array,
):
    B, C, H, W = x.shape
    R = H * W
    N = B * R
    assert B >= 4 and B % 2 == 0 and R % 128 == 0
    P = B // 2
    HL = R // (2 * _BLK)
    out_view = (P, 2, 2, HL, _BLK, C)

    tail = R * 5 // 8
    read_rows = (2 * R,) * (P - 1) + (2 * R - tail, tail)
    nr = len(read_rows)
    roff = [sum(read_rows[:i]) for i in range(nr)]
    wait_at = [off // R for off in roff]
    assert sum(read_rows) == N and wait_at[nr - 2:] == [B - 2, B - 1]

    def kernel(x_hbm, g_hbm, b_hbm, o_hbm, xbuf, obuf, gbuf, bbuf, sems):
        ins = [
            pltpu.make_async_copy(
                x_hbm.at[pl.ds(roff[i], read_rows[i])],
                xbuf.at[pl.ds(roff[i], read_rows[i])],
                sems.at[i % 2])
            for i in range(nr)
        ]
        copy_g = pltpu.make_async_copy(g_hbm, gbuf, sems.at[0])
        copy_b = pltpu.make_async_copy(b_hbm, bbuf, sems.at[0])
        out_sem = sems.at[(nr - 2) % 2]

        def write_out(*idx):
            pltpu.make_async_copy(obuf.at[idx], o_hbm.at[idx], out_sem).start()

        ins[0].start()
        copy_g.start()
        copy_b.start()
        ins[1].start()

        def normalize(bi):
            gamma = gbuf[...].astype(jnp.float32).reshape(1, C)
            beta = bbuf[...].astype(jnp.float32).reshape(1, C)
            base = pl.multiple_of(bi * R, R)
            xb = xbuf[pl.ds(base, R), :].astype(jnp.float32)
            mu = jnp.sum(xb, axis=0, keepdims=True) * (1.0 / R)
            d = xb - mu
            var = jnp.sum(d * d, axis=0, keepdims=True) * (1.0 / R)
            scale = jax.lax.rsqrt(var + _EPS) * gamma
            y = (d * scale + beta).astype(obuf.dtype)
            obuf[bi // 2, bi % 2] = y.reshape(2, HL, _BLK, C)

        def body(bi, carry):
            for i in range(nr):
                @pl.when(bi == wait_at[i])
                def _():
                    if i == 0:
                        copy_g.wait()
                        copy_b.wait()
                    ins[i].wait()
                    if i + 2 < nr:
                        ins[i + 2].start()
                    if i == nr - 2:
                        for p in range(2):
                            for hh in range(2):
                                for hl in range(HL):
                                    write_out(pl.ds(0, P - 1), p, hh, hl)
            normalize(bi)
            return carry

        jax.lax.fori_loop(0, B, body, 0)
        for hl in range(HL):
            write_out(P - 1, slice(None), slice(None), hl)
        pltpu.make_async_copy(obuf, o_hbm, out_sem).wait()

    xt = jnp.transpose(x, (0, 2, 3, 1)).reshape(N, C)
    out = pl.pallas_call(
        kernel,
        in_specs=[pl.BlockSpec(memory_space=pl.ANY)] * 3,
        out_specs=pl.BlockSpec(memory_space=pl.ANY),
        out_shape=jax.ShapeDtypeStruct(out_view, x.dtype),
        scratch_shapes=[
            pltpu.VMEM((N, C), x.dtype),
            pltpu.VMEM(out_view, x.dtype),
            pltpu.VMEM((C,), g.dtype),
            pltpu.VMEM((C,), b.dtype),
            pltpu.SemaphoreType.DMA((2,)),
        ],
        compiler_params=pltpu.CompilerParams(vmem_limit_bytes=64 * 1024 * 1024),
    )(xt, g, b)
    return jnp.transpose(out.reshape(B, H, W, C), (0, 3, 1, 2))
```
